```python
import os as _os
_os.environ.setdefault("JAX_PLATFORMS", "cpu")
import jax
import jax.numpy as jnp

def _softmax(x, axis=-1):
    return jax.nn.softmax(x, axis=axis)
def _gelu(x):
    return jax.nn.gelu(x, approximate=True)
def _silu(x):
    return jax.nn.silu(x)
def _sigmoid(x):
    return jax.nn.sigmoid(x)
def _layernorm(x, axis=-1, eps=1e-5):
    m = jnp.mean(x, axis=axis, keepdims=True)
    v = jnp.var(x, axis=axis, keepdims=True)
    return (x - m) / jnp.sqrt(v + eps)
def _scatter_add(tgt, idx, src, axis=0):
    return tgt.at[idx].add(src)
def _segment_sum(src, seg, n):
    return jax.ops.segment_sum(src, seg, n)
class _Rng:
    def __init__(self, key):
        self._k = key
    def _next(self):
        self._k, sub = jax.random.split(self._k)
        return sub
    def normal(self, shape):
        return jax.random.normal(self._next(), shape, dtype=jnp.bfloat16)
    def randint(self, lo, hi, shape):
        return jax.random.randint(self._next(), shape, lo, hi, dtype=jnp.int32)
    def uniform(self, shape, lo=0.0, hi=1.0):
        return jax.random.uniform(self._next(), shape, jnp.bfloat16, lo, hi)
    def permutation(self, n):
        return jax.random.permutation(self._next(), n)


kernel_name = 'standalone__sliding_block_cached__sampling'

def setup_inputs():
    _rng = _Rng(jax.random.key(int.from_bytes(__import__("os").urandom(4), "little")))
    _w = (lambda a: (lambda t: t.astype(jnp.bfloat16) if jnp.issubdtype(t.dtype, jnp.floating) else t)(jnp.asarray(a)))
    B, Sq, D = 8, 4, 640
    Hq, Hkv, Sk, Dh = 32, 32, 4096, 192
    assert Hq % Hkv == 0, (Hq, Hkv)
    return {
        "x": _w((lambda *s: _rng.normal(s) * 0.8)(B, Sq, D)),
        "k_cache": _w((lambda *s: _rng.normal(s) * 0.8)(B, Hkv, Sk, Dh)),
        "v_cache": _w((lambda *s: _rng.normal(s) * 0.05)(B, Hkv, Sk, Dh)),
        "wq": _w((lambda *s: _rng.normal(s) * 0.8)(D, Hq * Dh) * (D ** -0.5)),
        "wo": _w((lambda *s: _rng.normal(s) * 0.05)(Hq * Dh, D) * ((Hq * Dh) ** -0.5)),
    }

def reference(x, k_cache, v_cache, wq, wo):
    B, Sq, D = x.shape
    Hq, Dh = 32, 192
    Hkv, Sk = k_cache.shape[1], k_cache.shape[2]
    W = min(4096, max(256, Sk // 4))
    rep = Hq // Hkv
    q = (lambda x, *d: x.transpose(*d))((x @ wq).reshape(B, Sq, Hq, Dh), 0, 2, 1, 3)
    k = jnp.repeat(k_cache[:, :, Sk - W:, :], rep, axis=1)
    v = jnp.repeat(v_cache[:, :, Sk - W:, :], rep, axis=1)
    scores = jnp.einsum("bhqd,bhkd->bhqk", q, k) * (Dh ** -0.5)
    p = _softmax(scores, axis=-1)
    o = jnp.einsum("bhqk,bhkd->bhqd", p, v)
    return (lambda x, *d: x.transpose(*d))(o, 0, 2, 1, 3).reshape(B, Sq, Hq * Dh) @ wo
```

```python
import jax
import jax.numpy as jnp
from jax import lax
import jax.experimental.pallas as pl
import jax.experimental.pallas.tpu as pltpu

_NT = (((1,), (1,)), ((), ()))


@jax.jit
def pallas_standalone__sliding_block_cached__sampling_kernel(
    x: jax.Array,
    k_cache: jax.Array,
    v_cache: jax.Array,
    wq: jax.Array,
    wo: jax.Array,
):
    B, Sq, D = x.shape
    _, H, Sk, Dh = k_cache.shape
    W = min(4096, max(256, Sk // 4))
    assert Sk % W == 0
    HG, HPM = 8, 2
    NG = H // HG
    M = Sq * HPM
    KD = Dh * HPM
    GD = Dh * HG
    scale = Dh ** -0.5
    kt = jnp.swapaxes(k_cache, 2, 3).reshape(B, H * Dh, Sk)
    vt = jnp.swapaxes(v_cache, 2, 3).reshape(B, H * Dh, Sk)

    def kern(x_ref, wq_ref, wo_ref, k_ref, v_ref, out_ref, xd_ref, lhs_ref, o_ref, acc_ref):
        g = pl.program_id(0)
        b = pl.program_id(1)

        @pl.when((g == 0) & (b == 0))
        def _():
            for bb in range(B):
                xb = x_ref[bb].astype(jnp.float32)
                for j in range(HPM):
                    xd_ref[pl.ds(bb * M + j * Sq, Sq), :] = xb
            acc_ref[...] = jnp.zeros_like(acc_ref)

        @pl.when(b == 0)
        def _():
            q = jnp.dot(xd_ref[...].astype(jnp.bfloat16), wq_ref[...],
                        preferred_element_type=jnp.float32)
            row = (lax.broadcasted_iota(jnp.int32, q.shape, 0) % M) // Sq
            col = (lax.broadcasted_iota(jnp.int32, q.shape, 1) % KD) // Dh
            lhs_ref[...] = jnp.where(row == col, q * scale, 0.0).astype(jnp.bfloat16)

        r0 = pl.multiple_of(b * M, M)
        row = lax.broadcasted_iota(jnp.int32, (M, KD), 0) // Sq
        col = lax.broadcasted_iota(jnp.int32, (M, KD), 1) // Dh
        diag = row == col
        for mm in range(HG // HPM):
            lhs = lhs_ref[pl.ds(r0, M), mm * KD:(mm + 1) * KD]
            s = jnp.dot(lhs, k_ref[0, mm * KD:(mm + 1) * KD, :],
                        preferred_element_type=jnp.float32)
            m = jnp.max(s, axis=-1, keepdims=True)
            e = jnp.exp(s - m)
            l = jnp.sum(e, axis=-1, keepdims=True)
            o = lax.dot_general(e.astype(jnp.bfloat16), v_ref[0, mm * KD:(mm + 1) * KD, :],
                                _NT, preferred_element_type=jnp.float32)
            o = jnp.where(diag, o / l, 0.0)
            o_ref[pl.ds(r0, M), mm * KD:(mm + 1) * KD] = o.astype(jnp.bfloat16)

        @pl.when(b == B - 1)
        def _():
            acc_ref[...] += jnp.dot(o_ref[...], wo_ref[...],
                                    preferred_element_type=jnp.float32)

        @pl.when((g == NG - 1) & (b == B - 1))
        def _():
            for bb in range(B):
                r = acc_ref[pl.ds(bb * M, Sq), :]
                for j in range(1, HPM):
                    r = r + acc_ref[pl.ds(bb * M + j * Sq, Sq), :]
                out_ref[bb] = r.astype(out_ref.dtype)

    return pl.pallas_call(
        kern,
        grid=(NG, B),
        in_specs=[pl.BlockSpec((B, Sq, D), lambda g, b: (0, 0, 0)),
                  pl.BlockSpec((D, GD), lambda g, b: (0, g)),
                  pl.BlockSpec((GD, D), lambda g, b: (g, 0)),
                  pl.BlockSpec((1, GD, W), lambda g, b: (b, g, Sk // W - 1)),
                  pl.BlockSpec((1, GD, W), lambda g, b: (b, g, Sk // W - 1))],
        out_specs=pl.BlockSpec((B, Sq, D), lambda g, b: (0, 0, 0)),
        out_shape=jax.ShapeDtypeStruct((B, Sq, D), x.dtype),
        scratch_shapes=[pltpu.VMEM((B * M, D), jnp.float32),
                        pltpu.VMEM((B * M, GD), jnp.bfloat16),
                        pltpu.VMEM((B * M, GD), jnp.bfloat16),
                        pltpu.VMEM((B * M, D), jnp.float32)],
        compiler_params=pltpu.CompilerParams(
            dimension_semantics=("arbitrary", "arbitrary"),
            vmem_limit_bytes=100 * 1024 * 1024),
    )(x, wq, wo, kt, vt)
```

```python
import jax
import jax.numpy as jnp
from jax import lax
import jax.experimental.pallas as pl
import jax.experimental.pallas.tpu as pltpu

_NT = (((1,), (1,)), ((), ()))

_HG = 4
_HPM = 2
_NS = 3
_STRIDE = 37
_WO_ROWS = 32


def _unit_order(n_tiles, n_wq, n_wo):
    kv = []
    for i in range(n_tiles):
        t = (_STRIDE * i) % n_tiles
        kv += [("K", t, i % 2), ("V", t, i % 2)]
    a = [("WQ", j) for j in range(n_wq)]
    b = [("WO", j) for j in range(n_wo)]
    w = []
    while a or b:
        if a:
            w.append(a.pop(0))
        if b and len(b) * n_wq >= len(a) * n_wo:
            w.append(b.pop(0))
    n, m = len(kv), len(w)
    pos = [((2 * j + 1) * n) // (2 * m) // 4 * 4 for j in range(m)]
    out, wi = [], 0
    for i, d in enumerate(kv):
        while wi < m and pos[wi] == i:
            out.append((w[wi][0], w[wi][1], wi % 2))
            wi += 1
        out.append(d)
    assert wi == m
    return out


def _compiler_params():
    base = dict(vmem_limit_bytes=64 * 1024 * 1024)
    for extra in (dict(disable_bounds_checks=True, disable_semaphore_checks=True),
                  dict(disable_bounds_checks=True), dict()):
        try:
            return pltpu.CompilerParams(**base, **extra)
        except TypeError:
            continue
    return pltpu.CompilerParams(**base)


def _mult(v, m):
    return v if isinstance(v, int) else pl.multiple_of(v, m)


def _cond(c, fn):
    if isinstance(c, bool):
        if c:
            fn()
    else:
        pl.when(c)(fn)


def _spread(lo, hi, items):
    n = len(items)
    return [(round(lo + (hi - lo) * c / max(n - 1, 1)), it) for c, it in enumerate(items)]


def _run_interleaved(copies, placed):
    k = 0
    for i in range(len(copies) + 1):
        while k < len(placed) and placed[k][0] <= i:
            placed[k][1]()
            k += 1
        if i < len(copies):
            copies[i]()
    assert k == len(placed)


@jax.jit
def pallas_standalone__sliding_block_cached__sampling_kernel(
    x: jax.Array,
    k_cache: jax.Array,
    v_cache: jax.Array,
    wq: jax.Array,
    wo: jax.Array,
):
    B, Sq, D = x.shape
    _, H, Sk, Dh = k_cache.shape
    W = min(4096, max(256, Sk // 4))
    C0 = Sk - W
    NG = H // _HG
    M = Sq * _HPM
    KD = Dh * _HPM
    GD = Dh * _HG
    U = GD // 8
    NU = NG * B
    NP = _HG // _HPM
    WQ_PER = (D // 8) // B
    WO_PER = (GD // _WO_ROWS) // B
    scale = Dh ** -0.5
    assert wq.shape == (D, H * Dh) and wo.shape == (H * Dh, D)
    assert M == 8 and NP == 2 and GD % 128 == 0 and C0 % 128 == 0
    assert H % _HG == 0 and (D // 8) % B == 0 and (GD // _WO_ROWS) % B == 0
    order = _unit_order(U, WQ_PER, WO_PER)
    tail_pieces = ((0, KD), (KD, KD + 128), (KD + 128, KD + 256), (KD + 256, GD))

    kt = jnp.swapaxes(k_cache, 2, 3).reshape(B * H * Dh, Sk)
    vt = jnp.swapaxes(v_cache, 2, 3).reshape(B * H * Dh, Sk)

    def kernel(x_hbm, wq_hbm, wo_hbm, k_hbm, v_hbm, out_ref,
               kbuf, vbuf, wqbuf, wobuf, xbuf, xd_ref, lhs_ref, o_ref, acc_ref,
               ksem, vsem, wqsem, wosem, xsem):

        def wq_copy(g, rt):
            r = _mult(rt * 8, 8)
            return pltpu.make_async_copy(
                wq_hbm.at[pl.ds(r, 8), pl.ds(_mult(g * GD, 128), GD)],
                wqbuf.at[g % 2, pl.ds(r, 8)], wqsem.at[g % 2])

        def wo_copy(g, r, sem):
            r = _mult(r, 8)
            return pltpu.make_async_copy(
                wo_hbm.at[pl.ds(_mult(g * GD + r, 8), _WO_ROWS)],
                wobuf.at[g % 2, pl.ds(r, _WO_ROWS)], sem)

        def kv_copy(kind, u, slot, t, sem=None):
            r0 = _mult((u % B) * (H * Dh) + (u // B) * GD, 8)
            arr, buf, s = (k_hbm, kbuf, ksem) if kind == "K" else (v_hbm, vbuf, vsem)
            return pltpu.make_async_copy(
                arr.at[pl.ds(r0 + t * 8, 8), pl.ds(C0, W)],
                buf.at[slot, pl.ds(t * 8, 8)],
                s.at[slot] if sem is None else sem)

        def unit_copies(u, slot):
            g, b = u // B, u % B
            out = []
            for kind, t, pr in order:
                if kind in ("K", "V"):
                    def th(kind=kind, t=t, pr=pr):
                        kv_copy(kind, u, slot, t).start(priority=pr)
                elif kind == "WQ":
                    def th(t=t, pr=pr):
                        _cond(g + 1 < NG, lambda: wq_copy(
                            g + 1, b * WQ_PER + t).start(priority=pr))
                else:
                    def th(t=t, pr=pr):
                        _cond(g + 1 < NG, lambda: wo_copy(
                            g, (b * WO_PER + t) * _WO_ROWS, wosem.at[g % 2]).start(priority=pr))
                out.append(th)
            return out

        def wait_all(view, sem):
            pltpu.make_async_copy(view, view, sem).wait()

        row = lax.broadcasted_iota(jnp.int32, (M, KD), 0) // Sq
        col = lax.broadcasted_iota(jnp.int32, (M, KD), 1) // Dh
        diag = row == col

        def qproj(g):
            wait_all(wqbuf.at[g % 2], wqsem.at[g % 2])
            q = jnp.dot(xd_ref[...], wqbuf[g % 2], preferred_element_type=jnp.float32)
            rr = (lax.broadcasted_iota(jnp.int32, q.shape, 0) % M) // Sq
            cc = (lax.broadcasted_iota(jnp.int32, q.shape, 1) % KD) // Dh
            lhs_ref[...] = jnp.where(rr == cc, q * scale, 0.0).astype(jnp.bfloat16)

        def oproj(g):
            wait_all(wobuf.at[g % 2], wosem.at[g % 2])
            acc_ref[...] += jnp.dot(o_ref[...], wobuf[g % 2],
                                    preferred_element_type=jnp.float32)

        def qk_softmax(u, slot, p):
            r0 = _mult((u % B) * M, M)
            lhs = lhs_ref[pl.ds(r0, M), p * KD:(p + 1) * KD]
            s = jnp.dot(lhs, kbuf[slot, p * KD:(p + 1) * KD, :],
                        preferred_element_type=jnp.float32)
            m = jnp.max(s, axis=-1, keepdims=True)
            e = jnp.exp(s - m)
            l = jnp.sum(e, axis=-1, keepdims=True)
            return e.astype(jnp.bfloat16), l

        def pv(u, slot, p, e, l):
            r0 = _mult((u % B) * M, M)
            o = lax.dot_general(e, vbuf[slot, p * KD:(p + 1) * KD, :], _NT,
                                preferred_element_type=jnp.float32)
            o = jnp.where(diag, o / l, 0.0)
            o = o + pltpu.roll(o, Sq, 0)
            o_ref[pl.ds(r0, M), p * KD:(p + 1) * KD] = o.astype(jnp.bfloat16)

        def unit_pieces(u, slot):
            g, b = u // B, u % B
            st = {}

            def first():
                _cond(b == 0, lambda: qproj(g))
                wait_all(kbuf.at[slot], ksem.at[slot])
                wait_all(vbuf.at[slot], vsem.at[slot])

            pieces = [first]
            for p in range(NP):
                def p_qk(p=p):
                    st[p] = qk_softmax(u, slot, p)

                def p_pv(p=p):
                    pv(u, slot, p, *st[p])

                pieces += [p_qk, p_pv]
            pieces.append(lambda: _cond(b == B - 1, lambda: oproj(g)))
            return pieces

        xcp = pltpu.make_async_copy(x_hbm, xbuf, xsem.at[0])
        xcp.start()
        c0 = unit_copies(0, 0)
        nq = D // 8
        for j in range(nq):
            wq_copy(0, (j * 7) % nq).start(priority=j % 2)
            for th in c0[2 * j:2 * j + 2]:
                th()
        for th in c0[2 * nq:]:
            th()
        for u in range(1, _NS - 1):
            for th in unit_copies(u, u):
                th()
        xcp.wait()
        for bb in range(B):
            xb = xbuf[bb].astype(jnp.float32)
            for j in range(_HPM):
                acc_ref[pl.ds(bb * M + j * Sq, Sq), :] = xb
        xd_ref[...] = acc_ref[...].astype(jnp.bfloat16)
        acc_ref[...] = jnp.zeros_like(acc_ref)

        def body(i, carry):
            copies = unit_copies(i + _NS - 1, (i + _NS - 1) % _NS)
            pieces = unit_pieces(i, i % _NS)
            n = len(pieces)
            placed = [(round(len(copies) * (c + 1) / (n + 1)), pc)
                      for c, pc in enumerate(pieces)]
            _run_interleaved(copies, placed)
            return carry

        lax.fori_loop(0, NU - _NS, body, 0)

        uL, gL = NU - 1, NG - 1
        sL = uL % _NS
        h2 = U // 2
        copies = []
        for i in range(U):
            copies.append(lambda i=i: kv_copy("K", uL, sL, (11 * i) % U).start(priority=i % 2))
        for i in range(h2):
            copies.append(lambda i=i: kv_copy("V", uL, sL, (5 * i) % h2).start(priority=i % 2))
        for i in range(h2):
            copies.append(lambda i=i: kv_copy(
                "V", uL, sL, h2 + (5 * i) % h2, xsem.at[1]).start(priority=i % 2))
        for pi, (ra, rb) in enumerate(tail_pieces):
            for r in range(ra, rb, _WO_ROWS):
                copies.append(lambda r=r, pi=pi: wo_copy(
                    gL, r, xsem.at[2 + pi]).start(priority=1))
        placed = (_spread(8, U + 2, unit_pieces(uL - 2, (uL - 2) % _NS))
                  + _spread(U + 14, 2 * U - 4, unit_pieces(uL - 1, (uL - 1) % _NS)))
        _run_interleaved(copies, placed)

        wait_all(kbuf.at[sL], ksem.at[sL])
        el0 = qk_softmax(uL, sL, 0)
        el1 = qk_softmax(uL, sL, 1)
        wait_all(vbuf.at[sL, pl.ds(0, KD)], vsem.at[sL])
        pv(uL, sL, 0, *el0)
        wait_all(vbuf.at[sL, pl.ds(KD, KD)], xsem.at[1])
        pv(uL, sL, 1, *el1)
        a = acc_ref[...]
        for pi, (ra, rb) in enumerate(tail_pieces):
            wait_all(wobuf.at[gL % 2, pl.ds(ra, rb - ra)], xsem.at[2 + pi])
            a = a + jnp.dot(o_ref[:, ra:rb], wobuf[gL % 2, ra:rb, :],
                            preferred_element_type=jnp.float32)
        for bb in range(B):
            out_ref[bb] = a[bb * M:bb * M + Sq, :].astype(out_ref.dtype)

    hbm = pl.BlockSpec(memory_space=pl.ANY)
    return pl.pallas_call(
        kernel,
        in_specs=[hbm] * 5,
        out_specs=pl.BlockSpec((B, Sq, D), lambda: (0, 0, 0)),
        out_shape=jax.ShapeDtypeStruct((B, Sq, D), x.dtype),
        scratch_shapes=[
            pltpu.VMEM((_NS, GD, W), jnp.bfloat16),
            pltpu.VMEM((_NS, GD, W), jnp.bfloat16),
            pltpu.VMEM((2, D, GD), jnp.bfloat16),
            pltpu.VMEM((2, GD, D), jnp.bfloat16),
            pltpu.VMEM((B, Sq, D), jnp.bfloat16),
            pltpu.VMEM((B * M, D), jnp.bfloat16),
            pltpu.VMEM((B * M, GD), jnp.bfloat16),
            pltpu.VMEM((B * M, GD), jnp.bfloat16),
            pltpu.VMEM((B * M, D), jnp.float32),
            pltpu.SemaphoreType.DMA((_NS,)),
            pltpu.SemaphoreType.DMA((_NS,)),
            pltpu.SemaphoreType.DMA((2,)),
            pltpu.SemaphoreType.DMA((2,)),
            pltpu.SemaphoreType.DMA((2 + len(tail_pieces),)),
        ],
        compiler_params=_compiler_params(),
    )(x, wq, wo, kt, vt)
```

```python
import jax
import jax.numpy as jnp
from jax import lax
import jax.experimental.pallas as pl
import jax.experimental.pallas.tpu as pltpu

_NT = (((1,), (1,)), ((), ()))

_HG = 4
_HPM = 2
_AHEAD = 2
_STRIDE = 37
_WO_ROWS = 32


def _unit_order(n_tiles, n_wq, n_wo):
    kv = []
    for i in range(n_tiles):
        t = (_STRIDE * i) % n_tiles
        kv += [("K", t, i % 2), ("V", t, i % 2)]
    a = [("WQ", j) for j in range(n_wq)]
    b = [("WO", j) for j in range(n_wo)]
    w = []
    while a or b:
        if a:
            w.append(a.pop(0))
        if b and len(b) * n_wq >= len(a) * n_wo:
            w.append(b.pop(0))
    n, m = len(kv), len(w)
    pos = [((2 * j + 1) * n) // (2 * m) // 4 * 4 for j in range(m)]
    out, wi = [], 0
    for i, d in enumerate(kv):
        while wi < m and pos[wi] == i:
            out.append((w[wi][0], w[wi][1], wi % 2))
            wi += 1
        out.append(d)
    assert wi == m
    return out


def _compiler_params():
    base = dict(vmem_limit_bytes=64 * 1024 * 1024)
    for extra in (dict(disable_bounds_checks=True, disable_semaphore_checks=True),
                  dict(disable_bounds_checks=True), dict()):
        try:
            return pltpu.CompilerParams(**base, **extra)
        except TypeError:
            continue
    return pltpu.CompilerParams(**base)


def _mult(v, m):
    return v if isinstance(v, int) else pl.multiple_of(v, m)


def _cond(c, fn):
    if isinstance(c, bool):
        if c:
            fn()
    else:
        pl.when(c)(fn)


def _spread(lo, hi, items):
    n = len(items)
    return [(round(lo + (hi - lo) * c / max(n - 1, 1)), it) for c, it in enumerate(items)]


def _run_interleaved(copies, placed):
    k = 0
    for i in range(len(copies) + 1):
        while k < len(placed) and placed[k][0] <= i:
            placed[k][1]()
            k += 1
        if i < len(copies):
            copies[i]()
    assert k == len(placed)


@jax.jit
def pallas_standalone__sliding_block_cached__sampling_kernel(
    x: jax.Array,
    k_cache: jax.Array,
    v_cache: jax.Array,
    wq: jax.Array,
    wo: jax.Array,
):
    B, Sq, D = x.shape
    _, H, Sk, Dh = k_cache.shape
    W = min(4096, max(256, Sk // 4))
    C0 = Sk - W
    NG = H // _HG
    M = Sq * _HPM
    KD = Dh * _HPM
    GD = Dh * _HG
    U = GD // 8
    NP = _HG // _HPM
    PT = KD // 8
    WQ_PER = (D // 8) // B
    WO_PER = (GD // _WO_ROWS) // B
    scale = Dh ** -0.5
    assert wq.shape == (D, H * Dh) and wo.shape == (H * Dh, D)
    assert M == 8 and NP == 2 and GD % 128 == 0 and C0 % 128 == 0 and KD > 256
    assert H % _HG == 0 and (D // 8) % B == 0 and (GD // _WO_ROWS) % B == 0
    order = _unit_order(U, WQ_PER, WO_PER)
    tail_pieces = ((0, KD), (KD, KD + 128), (KD + 128, KD + 256), (KD + 256, GD))
    NKV = B * NP
    S_K, S_V, S_WQ, S_WO, S_X = 0, NKV, 2 * NKV, 2 * NKV + 2, 2 * NKV + 4
    S_T = S_X + 1
    NSEM = S_T + len(tail_pieces)

    kt = jnp.swapaxes(k_cache, 2, 3).reshape(B * H * Dh, Sk)
    vt = jnp.swapaxes(v_cache, 2, 3).reshape(B * H * Dh, Sk)

    def kernel(x_hbm, wq_hbm, wo_hbm, k_hbm, v_hbm, out_ref, *scratch):
        kbufs, vbufs = scratch[:NKV], scratch[NKV:2 * NKV]
        wqbuf, wobuf, xbuf, xd_ref, lhs_ref, o_ref, acc_ref, sems = scratch[2 * NKV:]

        def wq_copy(g, rt):
            return pltpu.make_async_copy(
                wq_hbm.at[pl.ds(rt * 8, 8), pl.ds(_mult(g * GD, 128), GD)],
                wqbuf.at[g % 2, pl.ds(rt * 8, 8)], sems.at[S_WQ + g % 2])

        def wo_copy(g, r, sem):
            return pltpu.make_async_copy(
                wo_hbm.at[pl.ds(_mult(g * GD + r, 8), _WO_ROWS)],
                wobuf.at[g % 2, pl.ds(r, _WO_ROWS)], sem)

        def kv_copy(kind, g, b, t):
            r0 = _mult(b * (H * Dh) + g * GD + t * 8, 8)
            arr, bufs, s0 = (k_hbm, kbufs, S_K) if kind == "K" else (v_hbm, vbufs, S_V)
            i = b * NP + t // PT
            return pltpu.make_async_copy(
                arr.at[pl.ds(r0, 8), pl.ds(C0, W)],
                bufs[i].at[pl.ds((t % PT) * 8, 8)], sems.at[s0 + i])

        def unit_copies(g, b, not_last):
            out = []
            for kind, t, pr in order:
                if kind in ("K", "V"):
                    def th(kind=kind, t=t, pr=pr):
                        kv_copy(kind, g, b, t).start(priority=pr)
                elif kind == "WQ":
                    def th(t=t, pr=pr):
                        _cond(not_last, lambda: wq_copy(
                            g + 1, b * WQ_PER + t).start(priority=pr))
                else:
                    def th(t=t, pr=pr):
                        _cond(not_last, lambda: wo_copy(
                            g, (b * WO_PER + t) * _WO_ROWS,
                            sems.at[S_WO + g % 2]).start(priority=pr))
                out.append(th)
            return out

        def wait_all(view, sem):
            pltpu.make_async_copy(view, view, sem).wait()

        row = lax.broadcasted_iota(jnp.int32, (M, KD), 0) // Sq
        col = lax.broadcasted_iota(jnp.int32, (M, KD), 1) // Dh
        diag = row == col

        def qproj(g):
            wait_all(wqbuf.at[g % 2], sems.at[S_WQ + g % 2])
            q = jnp.dot(xd_ref[...], wqbuf[g % 2], preferred_element_type=jnp.float32)
            rr = (lax.broadcasted_iota(jnp.int32, q.shape, 0) % M) // Sq
            cc = (lax.broadcasted_iota(jnp.int32, q.shape, 1) % KD) // Dh
            lhs_ref[...] = jnp.where(rr == cc, q * scale, 0.0).astype(jnp.bfloat16)

        def oproj(g):
            wait_all(wobuf.at[g % 2], sems.at[S_WO + g % 2])
            acc_ref[...] += jnp.dot(o_ref[...], wobuf[g % 2],
                                    preferred_element_type=jnp.float32)

        def qk_softmax(b, p):
            i = b * NP + p
            wait_all(kbufs[i], sems.at[S_K + i])
            lhs = lhs_ref[b * M:(b + 1) * M, p * KD:(p + 1) * KD]
            s = jnp.dot(lhs, kbufs[i][...], preferred_element_type=jnp.float32)
            m = jnp.max(s, axis=-1, keepdims=True)
            e = jnp.exp(s - m)
            l = jnp.sum(e, axis=-1, keepdims=True)
            return e.astype(jnp.bfloat16), l

        def pv(b, p, e, l):
            i = b * NP + p
            wait_all(vbufs[i], sems.at[S_V + i])
            o = lax.dot_general(e, vbufs[i][...], _NT, preferred_element_type=jnp.float32)
            o = jnp.where(diag, o / l, 0.0)
            o = o + pltpu.roll(o, Sq, 0)
            o_ref[b * M:(b + 1) * M, p * KD:(p + 1) * KD] = o.astype(jnp.bfloat16)

        def unit_pieces(g, b):
            st = {}
            pieces = [(lambda: qproj(g)) if b == 0 else (lambda: None)]
            for p in range(NP):
                def p_qk(p=p):
                    st[p] = qk_softmax(b, p)

                def p_pv(p=p):
                    pv(b, p, *st[p])

                pieces += [p_qk, p_pv]
            pieces.append((lambda: oproj(g)) if b == B - 1 else (lambda: None))
            return pieces

        def step(g, b, copies):
            pieces = unit_pieces(g, b)
            n = len(pieces)
            placed = [(round(len(copies) * (c + 1) / (n + 1)), pc)
                      for c, pc in enumerate(pieces)]
            _run_interleaved(copies, placed)

        xcp = pltpu.make_async_copy(x_hbm, xbuf, sems.at[S_X])
        xcp.start()
        c0 = unit_copies(0, 0, True)
        nq = D // 8
        for j in range(nq):
            wq_copy(0, (j * 7) % nq).start(priority=j % 2)
            for th in c0[2 * j:2 * j + 2]:
                th()
        for th in c0[2 * nq:]:
            th()
        for b in range(1, _AHEAD):
            for th in unit_copies(0, b, True):
                th()
        xcp.wait()
        for bb in range(B):
            xb = xbuf[bb].astype(jnp.float32)
            for j in range(_HPM):
                acc_ref[pl.ds(bb * M + j * Sq, Sq), :] = xb
        xd_ref[...] = acc_ref[...].astype(jnp.bfloat16)
        acc_ref[...] = jnp.zeros_like(acc_ref)

        def body(g, carry):
            for b in range(B):
                if b + _AHEAD < B:
                    copies = unit_copies(g, b + _AHEAD, g + 1 < NG)
                else:
                    copies = unit_copies(g + 1, b + _AHEAD - B, g + 2 < NG)
                step(g, b, copies)
            return carry

        lax.fori_loop(0, NG - 1, body, 0)

        gL, bL = NG - 1, B - 1
        for b in range(B - _AHEAD - 1):
            step(gL, b, unit_copies(gL, b + _AHEAD, False))

        copies = []
        for i in range(U):
            copies.append(lambda i=i: kv_copy("K", gL, bL, (11 * i) % U).start(priority=i % 2))
        for p in range(NP):
            for i in range(PT):
                copies.append(lambda i=i, p=p: kv_copy(
                    "V", gL, bL, p * PT + (5 * i) % PT).start(priority=i % 2))
        for pi, (ra, rb) in enumerate(tail_pieces):
            for r in range(ra, rb, _WO_ROWS):
                copies.append(lambda r=r, pi=pi: wo_copy(
                    gL, r, sems.at[S_T + pi]).start(priority=1))
        placed = (_spread(8, U + 2, unit_pieces(gL, bL - 2))
                  + _spread(U + 14, 2 * U - 4, unit_pieces(gL, bL - 1)))
        _run_interleaved(copies, placed)

        el = [qk_softmax(bL, p) for p in range(NP)]
        for p in range(NP):
            pv(bL, p, *el[p])
        a = acc_ref[...]
        for pi, (ra, rb) in enumerate(tail_pieces):
            wait_all(wobuf.at[gL % 2, pl.ds(ra, rb - ra)], sems.at[S_T + pi])
            a = a + jnp.dot(o_ref[:, ra:rb], wobuf[gL % 2, ra:rb, :],
                            preferred_element_type=jnp.float32)
        for bb in range(B):
            out_ref[bb] = a[bb * M:bb * M + Sq, :].astype(out_ref.dtype)

    hbm = pl.BlockSpec(memory_space=pl.ANY)
    return pl.pallas_call(
        kernel,
        in_specs=[hbm] * 5,
        out_specs=pl.BlockSpec((B, Sq, D), lambda: (0, 0, 0)),
        out_shape=jax.ShapeDtypeStruct((B, Sq, D), x.dtype),
        scratch_shapes=(
            [pltpu.VMEM((KD, W), jnp.bfloat16) for _ in range(2 * NKV)] + [
                pltpu.VMEM((2, D, GD), jnp.bfloat16),
                pltpu.VMEM((2, GD, D), jnp.bfloat16),
                pltpu.VMEM((B, Sq, D), jnp.bfloat16),
                pltpu.VMEM((B * M, D), jnp.bfloat16),
                pltpu.VMEM((B * M, GD), jnp.bfloat16),
                pltpu.VMEM((B * M, GD), jnp.bfloat16),
                pltpu.VMEM((B * M, D), jnp.float32),
                pltpu.SemaphoreType.DMA((NSEM,)),
            ]),
        compiler_params=_compiler_params(),
    )(x, wq, wo, kt, vt)
```
